```python
import os as _os
_os.environ.setdefault("JAX_PLATFORMS", "cpu")
import jax
import jax.numpy as jnp

def _softmax(x, axis=-1):
    return jax.nn.softmax(x, axis=axis)
def _gelu(x):
    return jax.nn.gelu(x, approximate=True)
def _silu(x):
    return jax.nn.silu(x)
def _sigmoid(x):
    return jax.nn.sigmoid(x)
def _layernorm(x, axis=-1, eps=1e-5):
    m = jnp.mean(x, axis=axis, keepdims=True)
    v = jnp.var(x, axis=axis, keepdims=True)
    return (x - m) / jnp.sqrt(v + eps)
def _scatter_add(tgt, idx, src, axis=0):
    return tgt.at[idx].add(src)
def _segment_sum(src, seg, n):
    return jax.ops.segment_sum(src, seg, n)
class _Rng:
    def __init__(self, key):
        self._k = key
    def _next(self):
        self._k, sub = jax.random.split(self._k)
        return sub
    def normal(self, shape):
        return jax.random.normal(self._next(), shape, dtype=jnp.bfloat16)
    def randint(self, lo, hi, shape):
        return jax.random.randint(self._next(), shape, lo, hi, dtype=jnp.int32)
    def uniform(self, shape, lo=0.0, hi=1.0):
        return jax.random.uniform(self._next(), shape, jnp.bfloat16, lo, hi)
    def permutation(self, n):
        return jax.random.permutation(self._next(), n)


kernel_name = 'interleave_layers__sliding_local_dilated__mixer_s_mlp__prompt'

def setup_inputs():
    _rng = _Rng(jax.random.key(int.from_bytes(__import__("os").urandom(4), "little")))
    _w = (lambda a: (lambda t: t.astype(jnp.bfloat16) if jnp.issubdtype(t.dtype, jnp.floating) else t)(jnp.asarray(a)))
    def _A_setup():
        B, S, D = 1, 2048, 448
        return {
            "x": _w((lambda *s: _rng.normal(s) * 0.05)(B, S, D)),
            "wqkv": _w((lambda *s: _rng.normal(s) * 0.05)(D, 3 * D)),
            "wo": _w((lambda *s: _rng.normal(s) * 0.05)(D, D)),
        }
    _A_in = _A_setup()

    def _B_setup():
        B, S, D, F = 1, 2048, 448, 1792
        return {
            "x":  _w((lambda *s: _rng.normal(s) * 0.05)(B, S, D)),
            "w1": _w((lambda *s: _rng.normal(s) * 0.8)(D, D) * (D ** -0.5)),
            "w2": _w((lambda *s: _rng.normal(s) * 0.8)(D, D) * (D ** -0.5)),
            "w3": _w((lambda *s: _rng.normal(s) * 0.8)(D, F) * (D ** -0.5)),
            "w4": _w((lambda *s: _rng.normal(s) * 0.8)(F, D) * (F ** -0.5)),
        }
    _B_in = _B_setup()

    return {
        "A_x": _A_in["x"],
        "A_wqkv": _A_in["wqkv"],
        "A_wo": _A_in["wo"],
        "B_x": _B_in["x"],
        "B_w1": _B_in["w1"],
        "B_w2": _B_in["w2"],
        "B_w3": _B_in["w3"],
        "B_w4": _B_in["w4"],
    }

def reference(A_x, A_wqkv, A_wo, B_x, B_w1, B_w2, B_w3, B_w4):
    def _A_ref(x, wqkv, wo):
        B, S, D = x.shape
        H = 16; Dh = D // H
        W, dil = 8, 2
        qkv = (lambda x, *d: x.transpose(*d))((x @ wqkv).reshape(B, S, 3, H, Dh), 2, 0, 3, 1, 4)
        q, k, v = qkv[0], qkv[1], qkv[2]
        scale = Dh ** -0.5
        pos = jnp.arange(S)
        off = jnp.arange(W) * dil
        idx = pos[:, None] - off[None, :]
        mask = idx >= 0
        idx_c = jnp.where(mask, idx, 0).reshape(-1)
        kg = k[:, :, idx_c, :].reshape(B, H, S, W, Dh)
        vg = v[:, :, idx_c, :].reshape(B, H, S, W, Dh)
        logits = jnp.einsum("bhsd,bhswd->bhsw", q, kg) * scale
        logits = jnp.where(mask[None, None, :, :], logits, -1e9)
        attn = _softmax(logits, axis=-1)
        o = jnp.einsum("bhsw,bhswd->bhsd", attn, vg)
        return (lambda x, *d: x.transpose(*d))(o, 0, 2, 1, 3).reshape(B, S, D) @ wo

    def _B_ref(x, w1, w2, w3, w4):
        B, S, D = x.shape
        h = _gelu(_layernorm(x, axis=-1) @ w1)
        c = D // 4
        g0 = jnp.pad(h[:, :, 0*c:1*c], ((0, 0), (1, 0), (0, 0)))[:, :S, :]
        g1 = jnp.pad(h[:, :, 1*c:2*c], ((0, 0), (0, 1), (0, 0)))[:, 1:, :]
        g2 = jnp.pad(h[:, :, 2*c:3*c], ((0, 0), (2, 0), (0, 0)))[:, :S, :]
        g3 = jnp.pad(h[:, :, 3*c:   ], ((0, 0), (0, 2), (0, 0)))[:, 2:, :]
        hs = jnp.concatenate([g0, g1, g2, g3], axis=-1) @ w2
        x1 = x + hs
        h2 = _gelu(_layernorm(x1, axis=-1) @ w3) @ w4
        return x1 + h2

    x = A_x
    x = x + _A_ref(_layernorm(x, axis=-1), A_wqkv, A_wo)
    x = x + _B_ref(_layernorm(x, axis=-1), B_w1, B_w2, B_w3, B_w4)
    x = x + _A_ref(_layernorm(x, axis=-1), A_wqkv, A_wo)
    x = x + _B_ref(_layernorm(x, axis=-1), B_w1, B_w2, B_w3, B_w4)
    return x
```

```python
import functools

import jax
import jax.numpy as jnp
import numpy as np
import jax.experimental.pallas as pl
import jax.experimental.pallas.tpu as pltpu

S, D, NH, DH, FF = 2048, 448, 16, 28, 1792
WIN = 8
NT = 16
LN = 128
HD = D // 2
CG = D // 4
EPS = 1e-5
F32, BF16, U32 = jnp.float32, jnp.bfloat16, jnp.uint32
GELU_C = float(np.sqrt(2.0 / np.pi))
GELU_A = 0.044715 * GELU_C
GELU_K = float(np.cbrt(GELU_A))

PAIRS = [(0, 2), (4, 6), (8, 10), (12, 14), (1, 3), (5, 7), (9, 11), (13, 15)]

NEIGHBOURS = [{n for n, q in enumerate(PAIRS) for j in p for o in (-2, -1, 1, 2) if (j + o) % NT in q} for p in PAIRS]

CFG = dict(only="", head="q0 q1 q2 q3 k0 k1 k2 k3 v0 v1 v2 v3 k4 k5 v4 v5 k6 v6 q4 k7 v7",
           mixo="o0 q5 o1 o2 q6 h0 q7 h1 h2 o4 o5 o3 h4 h5 h3 s1 o6 a1 b1 o7 c1 e1 h6 h7 s2 d1 s0",
           mlp0="g2 s3 d2 q1 k1 v1 g0 s4 d0 q2 k2 v2 g3 s5 d3 q0 k0 v0 g4 s6 d4 q3 k3 v3 g5 s7 d5 k4 v4 g6 k5 d6 v5 "
                "g7 k6 d7 v6 q4 k7 v7",
           mlp1="g2 s3 d2 g0 s4 d0 g3 s5 d3 g4 s6 d4 g5 s7 d5 g6 g7 d6 d7", ksplit=[7], xw=4, ew=0,
           nxc=8, opaque=0, u32="", free=["qkv", "wo", "w1"], ep=7, elag=4, hold=20, vp=2, np=7, nz=2, nlag=8, sp=2, slag=8, plain="xyzgqkvho", skew=3, rows=16, tie=1, groups=[0, 4, 7, 11], phase=0, lag=12, early=2,
           gain=1.25, floor=0.6, cap=2.0, horizon=600, prep_at={"3": 7, "o": 10, "1": 11, "4": 14, "2": 16}, flags={})


def _gelu_of_twice(z):
    return z * jnp.tanh(z * (z * z * (8 * GELU_A) + 2 * GELU_C)) + z


def _gelu_scaled(z):
    return z * jnp.tanh(z * (z * z + GELU_C / GELU_K)) + z


def _lhs_operands(a11, a12, a21, a22):
    return (a11 + a22, a21 + a22, a11, a22, a11 + a12, a21 - a11, a12 - a22)


def _rhs_operands(b11, b12, b21, b22):
    return (b11 + b22, b11, b12 - b22, b21 - b11, b22, b11 + b12, b21 + b22)


def _combine(m):
    m1, m2, m3, m4, m5, m6, m7 = m
    return (m1 + m4) + (m7 - m5), m3 + m5, m2 + m4, (m1 - m2) + (m3 + m6)


def _fold8(x):
    acc = x[0:8]
    for r in range(8, x.shape[0], 8):
        acc = acc + x[r:r + 8]
    return acc


def _mean(acc):
    return jnp.sum(acc, axis=0, keepdims=True) * (1.0 / D)


_RHS = (lambda b11, b12, b21, b22: b11 + b22, lambda b11, b12, b21, b22: b11, lambda b11, b12, b21, b22: b12 - b22,
        lambda b11, b12, b21, b22: b21 - b11, lambda b11, b12, b21, b22: b22, lambda b11, b12, b21, b22: b11 + b12,
        lambda b11, b12, b21, b22: b21 + b22)


def _job_order(cfg):
    def qkv(ps, layer, cs=(0, 1, 2)):
        return [("qkv", p, layer, c) for c in cs for p in ps]

    def mix(ps, layer):
        return [(k, p, layer) for k in ("wo", "w1") for p in ps]

    def mlp(ps, layer):
        return ([("w2", p, layer) for p in ps] + [("w3", p, layer, c) for p in ps for c in range(4)]
                + [("w4", p, layer) for p in ps])

    def mix_skewed(ps, layer):
        out = []
        for n in range(len(ps) + cfg["skew"]):
            if n < len(ps):
                out.append(("wo", ps[n], layer))
            if n >= cfg["skew"]:
                out.append(("w1", ps[n - cfg["skew"]], layer))
        return out

    only = cfg["only"]
    if only == "mlp" and not cfg.get("list"):
        return mlp((1, 2), 0) + qkv((1, 2), 1)
    if only == "mix":
        return mix_skewed(range(8), 0)
    def parse(text, layer, qkv_layer=None):
        out = []
        for word in text.split():
            kind, p = word[0], int(word[1])
            if kind in "qkv":
                out.append(("qkv", p, 1 if cfg.get("list") else qkv_layer or layer, "qkv".index(kind)))
            elif kind in "abce":
                out.append(("w3", p, layer, "abce".index(kind)))
            elif kind == "g":
                out += [("w3", p, layer, c) for c in range(4)]
            else:
                out.append(({"o": "wo", "h": "w1", "s": "w2", "d": "w4"}[kind], p, layer))
        return out

    if cfg.get("list"):
        return parse(cfg["list"].replace("_", " "), 0)
    jobs = parse(cfg["head"], 0)
    for layer in range(2):
        jobs += parse(cfg["mixo"], layer) + parse(cfg["mlp%d" % layer], layer, 1)
    if only == "head":
        jobs = jobs[:cfg.get("njobs", 32)]
    return jobs


def _pieces(task, cfg):
    big = [cfg["xw"]]
    if task[0] == "prep":
        return {"q": big + [1] * 14, "k": big + [1] * 14, "v": big + [1] * 14, "o": [1] * 4 + big + [1] * 14,
                "1": big + [1] * 14, "2": big + [1] * 14, "3": (big + [1] * 14) + (big + [1] * 14),
                "4": [2] * 14}[task[1]]
    norm = [1] * (cfg["vp"] + cfg["np"])
    return {"ln0": (big if task[1] < 4 else [1]) + norm, "norm": norm, "attn": [1] * 50,
            "shift": [1] * (2 * cfg["sp"])}.get(task[0], [0 if task[0] in cfg["free"] else 1] * cfg["ep"])


def _needs(item):
    kind, p, layer = item[:3]
    if kind == "qkv":
        return [("ln0", p) if layer == 0 else ("norm", p, 0, "w4"), ("prep", "qkv"[item[3]])]
    if kind == "attn":
        group = range(4) if p < 4 else range(4, 8)
        return ([("qkv", p, layer, 0)] + [("qkv", n, layer, c) for n in group for c in (1, 2)]
                + [("qkv", 0, layer, 2)])
    if kind == "wo":
        return [("attn", p, layer), ("prep", "o")]
    if kind == "w1":
        return [("norm", p, layer, "wo"), ("prep", "1")]
    if kind == "w2":
        return [("shift", p, layer), ("prep", "2")]
    if kind == "shift":
        return [("w1", n, layer) for n in sorted(NEIGHBOURS[p])]
    if kind == "w3":
        return [("norm", p, layer, "w2"), ("prep", "3")]
    return [("w3", p, layer, c) for c in range(4)] + [("prep", "4")]


def _plan(cfg):
    jobs = _job_order(cfg)
    points, first = [], {}
    count = 0
    for job in jobs:
        first[job] = len(points)
        for i in range(7):
            n = len(points)
            for t in range(FF // 2 // LN if job[0] == "w4" else 2):
                if count % 4 == cfg["phase"]:
                    points += [(job, i, t, g) for g in cfg["groups"]]
                count += 1
            if len(points) == n:
                points.append((job, i))
    end = len(points)
    after_job = dict(zip(jobs, [first[j] for j in jobs[1:]] + [end]))
    release, deadline, before = {}, {}, {}

    def visit(task, due):
        kind = task[0]
        if cfg["only"] in ("mlp", "mix") and (kind == "prep" or (kind == "attn" and task[1] < cfg.get("att0", 4))):
            return
        source = (task[3],) + task[1:3] if kind == "norm" else task
        if kind not in ("prep", "ln0", "attn", "shift") and source not in first:
            return
        if task not in deadline:
            before[task], release[task] = [], 0
            if kind in ("attn", "shift"):
                before[task] = [t for t in _needs(task) if t in first]
                release[task] = max([after_job[t] + cfg["lag"] for t in before[task]] + [0])
            elif kind == "norm":
                before[task], release[task] = [source], after_job[source] + cfg["nlag"]
            elif kind == "prep":
                before[task] = [("prep", "k")] if task[1] == "v" else []
                release[task] = first[jobs[cfg["prep_at"].get(task[1], 0)]]
            elif kind == "ln0":
                before[task] = [("ln0", task[1] - 4)] if task[1] >= 4 else []
            else:
                release[task] = after_job[task] + cfg["elag"]
                if kind == "qkv" and task[3] == 2 and task[1] != 0:
                    before[task] = [("qkv", 0, task[2], 2)]
        deadline[task] = min(deadline.get(task, end), due)
        for t in before[task]:
            visit(t, deadline[task] - int(sum(_pieces(task, cfg))))

    for job in jobs:
        for t in _needs(job):
            assert t not in first or first[t] < first[job], (job, t)
            visit(t, first[job] - cfg["early"])
    for job in jobs:
        visit(job, min(end, after_job[job] + cfg["hold"]))
    order = {t: n for n, t in enumerate(deadline)}
    left = {t: _pieces(t, cfg) for t in deadline}
    steps = []
    shared = [None]

    def staged(t):
        return t[0] == "prep" and t[1] in "qkvo"

    def ready(t, now):
        if staged(t) and shared[0] not in (None, t):
            return False
        return release[t] <= now and not any(left.get(b) for b in before[t])

    def emit(t, point):
        weight = left[t].pop(0)
        steps.append(("piece", t, point))
        if staged(t):
            shared[0] = t if left[t] else None
        return weight

    def force(t):
        for b in before[t] + ([shared[0]] if staged(t) and shared[0] not in (None, t) else []):
            if left.get(b):
                force(b)
        while left[t]:
            emit(t, None)

    if ("prep", "q") in left:
        force(("prep", "q"))
    if cfg["only"] not in ("mlp", "mix"):
        steps.append(("x_in",))
    credit = 0.0
    for now, point in enumerate(points):
        job, i = point[:2]
        if now == first[job]:
            for need in _needs(job):
                if left.get(need):
                    if cfg.get("verbose"):
                        print("forced", need, sum(left[need]), "before", job)
                    force(need)
        if len(point) == 2:
            steps.append(("dot", job, i))
            continue
        todo = sorted((t for t in left if left[t]), key=lambda t: (deadline[t], order[t]))
        rate, work = 0.0, 0
        for t in todo:
            work += sum(left[t])
            if deadline[t] - now <= cfg["horizon"]:
                rate = max(rate, work / max(deadline[t] - now, 1))
        rate = min(max(rate * cfg["gain"], cfg["floor"]), cfg["cap"])
        credit += rate
        while True:
            t = next((t for t in todo if left[t] and ready(t, now)), None)
            if t is None:
                credit = min(credit, 1.0)
                break
            if credit < left[t][0]:
                break
            credit -= emit(t, point)
        if cfg.get("verbose") and now == first[job]:
            print(job, "rate %.2f" % rate)
        if now + 1 == end or points[now + 1][:2] != (job, i):
            steps.append(("dot", job, i))
    for t in sorted(left, key=lambda t: (deadline[t], order[t])):
        if left[t]:
            force(t)
    return steps


_SLOTS = dict(x=NT, y=NT, z=NT, q=NT, k=2 * NT, v=2 * NT, h=NT + 4, o=NT, g=32, p=8, lq=11, lo=4, l1=4, l2=4, l3=14, l4=13)
_BASE = dict(zip(_SLOTS, np.cumsum([0] + list(_SLOTS.values()))[:-1].tolist()))
_NSLOT = sum(_SLOTS.values())


def _kernel(zero_ref, x_hbm, wqkv_hbm, wo_hbm, w1_hbm, w2_hbm, w3_hbm, w4_hbm, o_hbm,
            x_raw, wqkv_raw, wo_raw, w1_raw, w2_raw, w3_raw, w4_raw, o_raw,
            perm, tr, arena, sem_in, sem_out, *, cfg):
    rows = cfg["rows"]
    nv = rows // 8
    zero = zero_ref[0]
    lane = jax.lax.broadcasted_iota(jnp.int32, (8, LN), 1)

    def lane_is(i, n):
        return jnp.broadcast_to((lane == i)[None], (n // 8, 8, LN)).reshape(n, LN)

    values = {}

    def ld(name, j, r=pl.ds(0, D)):
        if name not in cfg["plain"] or (name, j) not in values:
            return pltpu.bitcast(arena[_BASE[name] + j, r, :], F32)
        lo, hi, parts = r.start, r.start + r.size, []
        for at, v in sorted(values[name, j].items()):
            a, b = max(lo, at), min(hi, at + v.shape[0])
            if a < b:
                parts.append(v if b - a == v.shape[0] else v[a - at:b - at])
        return parts[0] if len(parts) == 1 else jnp.concatenate(parts, axis=0)

    def st(name, j, r, v):
        if name in cfg["plain"]:
            if (name, j) not in values and cfg["only"] in ("mlp", "mix") and name == "x":
                values[name, j] = {q.start: ld(name, j, q) for sl in chunks for q in halves(sl)}
            values.setdefault((name, j), {})[r.start] = v
        else:
            arena[_BASE[name] + j, r, :] = pltpu.bitcast(v, U32)

    chunks = [slice(r, r + rows) for r in range(0, HD, rows)]

    def halves(sl):
        return pl.ds(sl.start, rows), pl.ds(HD + sl.start, rows)

    nxc = cfg["nxc"]
    xw = S // nxc
    x_cp = [pltpu.make_async_copy(x_hbm.at[:, pl.ds(c * xw, xw)], x_raw.at[:, pl.ds(c * xw, xw)],
                                  sem_in.at[c]) for c in range(nxc)]
    head = pl.ds(0, 4 * LN)
    tail = pl.ds(4 * LN, 3 * D - 4 * LN)
    w_cp = {n: pltpu.make_async_copy(src, dst, sem_in.at[nxc + i]) for i, (n, src, dst) in enumerate((
        ("q", wqkv_hbm.at[:, head], wqkv_raw.at[:, head]), ("kv", wqkv_hbm.at[:, tail], wqkv_raw.at[:, tail]),
        ("o", wo_hbm, wo_raw), ("1", w1_hbm, w1_raw),
        ("2", w2_hbm, w2_raw), ("3", w3_hbm, w3_raw), ("4", w4_hbm, w4_raw)))}
    o_cp = [pltpu.make_async_copy(o_raw.at[:, pl.ds(c * xw, xw)], o_hbm.at[:, pl.ds(c * xw, xw)],
                                  sem_out.at[c]) for c in range(nxc)]

    def lhs_place(name, unit):
        return _BASE[name] + unit // 4, (unit % 4) * (HD // 2)

    zero_bits = jnp.full((8, LN), zero, jnp.int32).astype(U32)

    def bits(v):
        return pltpu.bitcast(v[:8, :LN], U32)

    def after(word, results):
        return word | (functools.reduce(jnp.bitwise_or, results) & zero_bits)[:, :word.shape[1]]

    def put_lhs(name, c, r, n, a11, a12, a21, a22):
        if cfg.get("noprep"):
            return []
        if r // HD != (r + n - 1) // HD:
            k = HD - r % HD
            put_lhs(name, c, r, k, a11[:k], a12[:k], a21[:k], a22[:k])
            return put_lhs(name, c, r + k, n - k, a11[k:], a12[k:], a21[k:], a22[k:])
        c, r = c + r // HD, r % HD
        done = []
        nk = pl.cdiv(a11.shape[1], LN)
        for i, v in enumerate(_lhs_operands(a11, a12, a21, a22)):
            u = pltpu.bitcast(v.astype(BF16), U32)
            for t in range(nk):
                slot, r0 = lhs_place(name, (c * 7 + i) * nk + t)
                w = min(LN, u.shape[1] - t * LN)
                arena[slot, pl.ds(r0 + r // 2, n // 2), pl.ds(0, w)] = u[:, t * LN:t * LN + w]
            if i in (5, 6):
                done.append(u[:8, :LN])
        return done

    def lhs_tiles(name, c, i, kdim):
        nk = pl.cdiv(kdim, LN)
        return [lhs_place(name, (c * 7 + i) * nk + t) + (pl.ds(0, min(LN, kdim - t * LN)),) for t in range(nk)]

    def get_lhs(name, c, i, kdim, ties, shift):
        cols = []
        for t, (slot, r0, w) in enumerate(lhs_tiles(name, c, i, kdim)):
            slot = slot + shift
            parts, r = [], 0
            for g in sorted(g for tt, g in ties if tt == t):
                if 8 * g > r:
                    parts.append(arena[slot, pl.ds(r0 + r, 8 * g - r), w])
                parts.append(after(arena[slot, pl.ds(r0 + 8 * g, 8), w], ties[t, g]))
                r = 8 * g + 8
            if r < HD // 2:
                parts.append(arena[slot, pl.ds(r0 + r, HD // 2 - r), w])
            cols.append(jnp.concatenate(parts, axis=0))
        return pltpu.bitcast(jnp.concatenate(cols, axis=1), BF16)

    def transposed(raw, col, n):
        return [raw[pl.ds(h * HD, HD), pl.ds(col, n)].T.astype(F32) for h in range(2)]

    def stage(h, off, t):
        perm[2 * h, pl.ds(off, t.shape[0]), :] = t[:, :LN]
        perm[2 * h + 1, pl.ds(off, t.shape[0]), pl.ds(0, HD - LN)] = t[:, LN:]

    def perm_rows(h, idx):
        return jnp.concatenate([perm[2 * h, idx, :], perm[2 * h + 1, idx, :][:, :HD - LN]], axis=1)

    def prep_qkv(c):
        for b in ((0, 1, 2, 3), (4, 5, 6), (7, 8, 9, 10))[c]:
            t = transposed(wqkv_raw, b * LN, min(LN, 3 * D - b * LN))
            for h in range(2):
                stage(h, b * LN, t[h])
        yield [bits(v[-8:]) for v in t]
        for d in range(DH // 2):
            top, bot = (pl.ds(c * D + dd, NH, stride=DH) for dd in (d, d + DH // 2))
            yield put_lhs("lq", c, d * NH, NH, perm_rows(0, top), perm_rows(1, top), perm_rows(0, bot),
                          perm_rows(1, bot))

    def put_halves(name, k):
        for r in range(0, HD, 16):
            yield put_lhs(name, 0, r, 16, k[0][r:r + 16], k[1][r:r + 16], k[0][HD + r:HD + r + 16],
                          k[1][HD + r:HD + r + 16])

    def prep_o():
        for c in range(4):
            n = min(LN, D - c * LN)
            w = wo_raw[:, pl.ds(c * LN, n)].astype(F32)
            perm[c, pl.ds(0, D), pl.ds(0, n)] = w
            yield [bits(w[-8:])] if n == LN else []
        k = [[], []]
        for c in range(4):
            for h in range(2):
                blk = jnp.concatenate([perm[c, pl.ds(d, NH, stride=DH), :]
                                       for d in range(h * DH // 2, (h + 1) * DH // 2)], axis=0)
                k[h].append(blk[:, :min(LN, D - c * LN)].astype(BF16).T.astype(F32))
        yield [bits(v[-8:]) for half in k for v in half]
        yield from put_halves("lo", [jnp.concatenate(v, axis=0) for v in k])

    def prep_dd(raw, name):
        k = []
        for b in range(4):
            k.append(transposed(raw, b * LN, min(LN, D - b * LN)))
        yield [bits(v[-8:]) for pair in k for v in pair]
        yield from put_halves(name, [jnp.concatenate([v[h] for v in k], axis=0) for h in range(2)])

    def prep_3():
        k = []
        for first, last, rows_from, rows_to in ((0, 4, 0, 2 * HD), (4, 7, 2 * HD, 4 * HD)):
            k += [transposed(w3_raw, b * LN, LN) + transposed(w3_raw, FF // 2 + b * LN, LN) for b in range(first, last)]
            yield [bits(v[-8:]) for quad in k[first:] for v in quad]
            for r in range(rows_from, rows_to, 32):
                yield put_lhs("l3", 0, r, 32, *[v[r % LN:r % LN + 32] for v in k[r // LN]])

    def prep_4():
        for r in range(0, HD, 16):
            top, bot = (w4_raw[pl.ds(o + r, 16), :].astype(F32) for o in (0, HD))
            yield put_lhs("l4", 0, r, 16, top[:, :FF // 2], top[:, FF // 2:], bot[:, :FF // 2], bot[:, FF // 2:])

    spans = [(c * LN, min(LN, D - c * LN)) for c in range(4)]

    def x_in(c):
        x_cp[c].wait()
        for t in range(c * xw // LN, (c + 1) * xw // LN):
            for f, (r, n) in enumerate(spans):
                blk = x_raw[pl.ds(r, n), pl.ds(t * LN, LN)]
                if n < LN:
                    blk = jnp.concatenate([blk, jnp.zeros((LN - n, LN), BF16)], axis=0)
                tr[f, pl.ds(t * LN // 2, LN // 2), :] = pltpu.bitcast(blk.T, U32)

    def x_tiles(u):
        w = jnp.concatenate([tr[f, pl.ds(u, LN, stride=NT // 2), :].T[:n] for f, (_, n) in enumerate(spans)], axis=0)
        return pltpu.bitcast(w << 16, F32), pltpu.bitcast(w & np.uint32(0xFFFF0000), F32)

    finished = {}

    def out_tile(j):
        finished[j] = pltpu.bitcast(ld("x", j).astype(BF16).astype(F32), U32)
        if j ^ 1 in finished:
            w = (finished.pop(j & ~1) >> 16) | finished.pop(j | 1)
            for f, (r, n) in enumerate(spans):
                blk = w[r:r + n]
                if n < LN:
                    blk = jnp.concatenate([blk, jnp.zeros((LN - n, LN), U32)], axis=0)
                tr[f, pl.ds(j // 2, LN, stride=NT // 2), :] = blk.T

    def x_out(c):
        for t in range(c * xw // LN, (c + 1) * xw // LN):
            for f, (r, n) in enumerate(spans):
                blk = pltpu.bitcast(tr[f, pl.ds(t * LN // 2, LN // 2), :], BF16).T
                o_raw[pl.ds(r, n), pl.ds(t * LN, LN)] = blk[:n]
        o_cp[c].start()

    def quad(p, sl):
        a, b = PAIRS[p]
        top, bot = halves(sl)
        return (a, top), (b, top), (a, bot), (b, bot)

    operand_rows, operands_of = {}, {}

    def put_rhs(key, r, total, quadrants):
        rows_of = operand_rows.setdefault(key, {})
        rows_of[r] = _rhs_operands(*quadrants)
        done = [bits(rows_of[r][2][-8:]), bits(rows_of[r][3][-8:])]
        words = key[0] in cfg["u32"]
        if words:
            rows_of[r] = [pltpu.bitcast(v.astype(BF16), U32) for v in rows_of[r]]
            done = [rows_of[r][2][-8:], rows_of[r][3][-8:]]
        if sum(v[0].shape[0] for v in rows_of.values()) * (2 if words else 1) == total:
            whole = [jnp.concatenate([rows_of[k][i] for k in sorted(rows_of)], axis=0) for i in range(7)]
            operands_of[key] = [pltpu.bitcast(v, BF16) if words else v.astype(BF16) for v in whole]
            if key[0] == "g":
                cuts = np.cumsum([0] + cfg["ksplit"]) * LN
                operands_of[key] = [[v[a:b].astype(BF16) for a, b in zip(cuts[:-1], cuts[1:])] for v in whole]
            del operand_rows[key]
        return done

    def accumulate(sums, i, v):
        s = _fold8(v)
        sums[i % 2] = s if sums[i % 2] is None else sums[i % 2] + s

    def normalise(src, p, sums, gain, dst, keep=None):
        mean = [_mean(v) for v in sums]
        acc = [None, None]
        for n in range(cfg["vp"]):
            for sl in chunks[n * len(chunks) // cfg["vp"]:(n + 1) * len(chunks) // cfg["vp"]]:
                for i, (j, r) in enumerate(quad(p, sl)):
                    xc = ld(src, j, r) - mean[i % 2]
                    accumulate(acc, i, xc * xc)
            yield [bits(v) for v in acc]
        var = [_mean(v) for v in acc]
        rstd = [jax.lax.rsqrt(v + EPS) for v in var]
        if keep is not None:
            keep[p] = (mean, rstd)
        scale = [gain(v, r) for v, r in zip(var, rstd)]
        for n in range(cfg["np"]):
            done = []
            for sl in chunks[n * len(chunks) // cfg["np"]:(n + 1) * len(chunks) // cfg["np"]]:
                z = [(ld(src, j, r) - mean[i % 2]) * scale[i % 2] for i, (j, r) in enumerate(quad(p, sl))]
                done += put_rhs((dst, p), sl.start, HD, z)
            yield done[-cfg["nz"]:]

    def first_ln(p):
        sums = [None, None]
        for i, j in enumerate(PAIRS[p]):
            if j % 2 == 0:
                for tile, x in enumerate(x_tiles(j // 2)):
                    for sl in chunks:
                        for r in halves(sl):
                            st("x", j + tile, r, x[r.start:r.start + rows])
            accumulate(sums, i, ld("x", j))
        yield [bits(v) for v in sums]
        yield from normalise("x", p, sums, lambda var, rstd: rstd, "n")

    def pieces(kind):
        n = cfg["ep"]
        return [chunks[i * len(chunks) // n:(i + 1) * len(chunks) // n] for i in range(n)]

    def qkv_epi(p, c, m):
        for piece in pieces("qkv"):
            for sl in piece:
                out = _combine(m(sl))
                for (j, r), t in zip(quad(p, sl), out):
                    par, i = j % 2, j // 2
                    if c == 0:
                        st("q", j, r, t)
                        continue
                    name = "k" if c == 1 else "v"
                    st(name, par * NT + 8 + i, r, t)
                    if i > 0:
                        prev = pltpu.roll(t, 1, 1)
                        if c == 2:
                            prev = jnp.where(lane_is(0, rows), ld("v", 8, r), prev)
                        st(name, par * NT + i, r, prev)
            yield [bits(out[0][-8:]), bits(out[3][-8:])]

    def attn(p):
        a, _ = PAIRS[p]
        par, m = a % 2, a // 2
        first = par * NT + m + 1
        w = {}
        for hb in range(2):
            logit = {}
            for i in range(WIN + 1):
                use = [t for t in range(2) if 0 <= i - t < WIN]
                acc = {}
                for d in range(DH):
                    r = pl.ds(d * NH + hb * 8, 8)
                    k = ld("k", first + i, r)
                    for t in use:
                        prod = ld("q", a + 2 * t, r) * k
                        acc[t] = acc[t] + prod if d else prod
                for t in use:
                    lg = acc[t] * (DH ** -0.5)
                    logit[t, i - t] = jnp.where(lane == 0, -1e9, lg) if m + 1 + i < 8 else lg
                yield [bits(acc[t]) for t in use]
            for t in range(2):
                lg = [logit[t, i] for i in range(WIN)]
                peak = functools.reduce(jnp.maximum, lg)
                e = [jnp.exp(v - peak) for v in lg]
                inv = 1.0 / functools.reduce(jnp.add, e)
                w[t, hb] = [v * inv for v in e]
                yield [bits(inv)]
        for d in range(DH // 2):
            out = []
            for hb in range(2):
                out.append([])
                for dd in (d, d + DH // 2):
                    r = pl.ds(dd * NH + hb * 8, 8)
                    v = [ld("v", first + i, r) for i in range(WIN + 1)]
                    for t in range(2):
                        out[hb].append(functools.reduce(jnp.add, [w[t, hb][i] * v[i + t] for i in range(WIN)]))
                if hb == 0:
                    yield [bits(v) for v in out[0][1:3]]
            yield put_rhs(("o", p), d * NH, HD, [jnp.concatenate(v, axis=0) for v in zip(*out)])

    def shift(p):
        a, b = PAIRS[p]
        for g, (near, far) in enumerate(((-1, -2), (1, 2))):
            for n in range(cfg["sp"]):
                done = []
                for r in range(g * CG + CG // 16 * n // cfg["sp"] * 16, g * CG + CG // 16 * (n + 1) // cfg["sp"] * 16, 16):
                    top, bot = pl.ds(r, 16), pl.ds(HD + r, 16)
                    done += put_rhs(("h", p), r, HD, [ld("h", a + 2 + near, top), ld("h", b + 2 + near, top),
                                                      ld("h", a + 2 + far, bot), ld("h", b + 2 + far, bot)])
                yield done[-cfg["nz"]:]

    stats = {}
    if cfg["only"] == "mlp":
        stats = {p: ([ld("p", p, pl.ds(0, 8))[:1]] * 2, [ld("p", p, pl.ds(8, 8))[:1]] * 2) for p in range(8)}

    pending = {}

    def residual(p, m):
        sums = [None, None]
        for piece in pieces("res"):
            for sl in piece:
                for i, ((j, r), t) in enumerate(zip(quad(p, sl), m(sl))):
                    x = ld("x", j, r) + t
                    st("x", j, r, x)
                    accumulate(sums, i, x)
            yield sums

    def wo_epi(p, m):
        for sums in residual(p, lambda sl: _combine(m(sl))):
            pending[p, "wo"] = normalise(
                "x", p, sums, lambda var, rstd: 0.5 * rstd * jax.lax.rsqrt(var * rstd * rstd + EPS), "y", stats)
            yield [bits(v) for v in sums]

    def w1_epi(p, m):
        halos = {15: (1, 1, (0, 2)), 14: (0, 1, (2,)), 0: (18, -1, (1, 3)), 1: (19, -1, (3,))}
        for piece in pieces("w1"):
            done = []
            for sl in piece:
                for (j, r), t in zip(quad(p, sl), _combine(m(sl))):
                    h = _gelu_of_twice(t)
                    st("h", j + 2, r, h)
                    done.append(bits(h[-8:]))
                    slot, by, groups = halos.get(j, (0, 0, ()))
                    if r.start // CG in groups:
                        st("h", slot, r, jnp.where(lane_is(0 if by > 0 else LN - 1, rows), 0.0,
                                                   pltpu.roll(h, by % LN, 1)))
            yield done[-4:]

    def w2_epi(p, m):
        sums = [None, None]
        for piece in pieces("w2"):
            for sl in piece:
                for i, ((j, r), t) in enumerate(zip(quad(p, sl), _combine(m(sl)))):
                    x = ld("x", j, r)
                    x1 = (x - stats[p][0][i % 2]) * stats[p][1][i % 2] + t
                    st("y", j, r, x1)
                    st("x", j, r, x + x1)
                    accumulate(sums, i, x1)
            pending[p, "w2"] = normalise("y", p, sums, lambda var, rstd: GELU_K * rstd, "z")
            yield [bits(v) for v in sums]

    def w3_epi(p, c, m):
        for piece in pieces("w3"):
            for sl in piece:
                done = put_rhs(("g", p), c * HD + sl.start, FF // 2, [_gelu_scaled(t) for t in _combine(m(sl))])
            yield done

    def w4_epi(p, last, m):
        for n, sums in enumerate(residual(p, lambda sl: [v * (0.5 / GELU_K) for v in _combine(m(sl))])):
            if not last:
                pending[p, "w4"] = normalise("x", p, sums, lambda var, rstd: rstd, "n")
                yield [bits(v) for v in sums]
                continue
            if n + 1 == cfg["ep"]:
                for j in PAIRS[p]:
                    out_tile(j)
            yield []

    def waited(name, gen):
        w_cp[name].wait()
        yield from gen

    products, ties, running = {}, {}, {}
    njob = [0, 0]

    def start(task):
        kind, p = task[0], task[1]
        if kind == "prep":
            return {"q": lambda: waited("q", prep_qkv(0)), "k": lambda: waited("kv", prep_qkv(1)),
                    "v": lambda: prep_qkv(2), "o": lambda: waited("o", prep_o()),
                    "1": lambda: waited("1", prep_dd(w1_raw, "l1")), "2": lambda: waited("2", prep_dd(w2_raw, "l2")),
                    "3": lambda: waited("3", prep_3()), "4": lambda: waited("4", prep_4())}[p]()
        if kind == "norm":
            return pending.pop((p, task[3]))
        if task in products:
            return epilogue(task)
        return {"ln0": first_ln, "attn": attn, "shift": shift}[kind](p)

    def epilogue(job):
        kind, p = job[0], job[1]
        m = products.pop(job)
        get = lambda sl: [v[sl] for v in m]
        if kind == "qkv":
            return qkv_epi(p, job[3], get)
        if kind == "w3":
            return w3_epi(p, job[3], get)
        if kind == "w4":
            return w4_epi(p, job[2] == 1, get)
        return {"wo": wo_epi, "w1": w1_epi, "w2": w2_epi}[kind](p, get)

    def operands(job):
        kind, p = job[0], job[1]
        lhs = {"qkv": "lq", "wo": "lo", "w1": "l1", "w2": "l2", "w3": "l3", "w4": "l4"}[kind]
        return lhs, (job[3] if len(job) > 3 else 0), (FF // 2 if kind == "w4" else HD)

    def rhs(job, i):
        key = ({"w2": "h", "w4": "g", "wo": "o", "w1": "y", "w3": "z", "qkv": "n"}[job[0]], job[1])
        if key not in operands_of:
            put_rhs(key, 0, HD, [ld("p", n, pl.ds(0, HD)) for n in range(4)])
        return operands_of[key][i]

    if cfg["only"] not in ("mlp", "mix"):
        w_cp["q"].start()
        for cp in x_cp:
            cp.start()
    for step in _plan(cfg):
        if step[0] == "x_in":
            for c in range(nxc):
                x_in(c)
            for n in ("kv", "3", "o", "1", "4", "2"):
                w_cp[n].start()
        elif step[0] == "piece":
            _, task, point = step
            if task not in running:
                running[task] = start(task)
            results = next(running[task])
            if point is not None and results and cfg["tie"] and task[0] not in cfg["free"]:
                ties.setdefault(point[:2], {}).setdefault(point[2:], []).extend(results)
        else:
            _, job, i = step
            lhs, c, kdim = operands(job)
            if i == 0 and cfg["opaque"]:
                njob[0] += 1
                njob[1] = zero_ref[njob[0] % cfg["opaque"]]
            w = get_lhs(lhs, c, i, kdim, ties.pop((job, i), {}), njob[1])
            cuts = np.cumsum([0] + cfg["ksplit"]) * LN if job[0] == "w4" else [0, kdim]
            parts = [jnp.dot(w[:, a:b], rhs(job, i) if job[0] != "w4" else rhs(job, i)[n],
                             preferred_element_type=F32) for n, (a, b) in enumerate(zip(cuts[:-1], cuts[1:]))]
            products.setdefault(job, []).append(functools.reduce(jnp.add, parts))
    for gen in running.values():
        assert next(gen, None) is None
    if cfg["only"]:
        sink = [v[:16] for (name, _), part in values.items() if name in "xhqkv" for v in part.values()]
        for n, v in enumerate(sink):
            arena[_BASE["x"] + n // 20, pl.ds(n % 20 * 16, v.shape[0]), :] = pltpu.bitcast(v, U32)
        o_raw[0:16, 0:LN] = pltpu.bitcast(arena[zero, 0:8, :], BF16)
        o_cp[0].start()
        o_cp[0].wait()
        return
    for c in range(nxc):
        x_out(c)
    for cp in o_cp:
        cp.wait()


def build(cfg):
    def run(A_x, A_wqkv, A_wo, B_x, B_w1, B_w2, B_w3, B_w4):
        del B_x
        vm = pltpu.VMEM
        out = pl.pallas_call(
            functools.partial(_kernel, cfg=cfg),
            out_shape=jax.ShapeDtypeStruct((D, S), BF16),
            in_specs=[pl.BlockSpec(memory_space=pltpu.SMEM)] + [pl.BlockSpec(memory_space=pl.ANY)] * 7,
            out_specs=pl.BlockSpec(memory_space=pl.ANY),
            scratch_shapes=[
                vm((D, S), BF16), vm((D, 3 * D), BF16), vm((D, D), BF16), vm((D, D), BF16), vm((D, D), BF16),
                vm((D, FF), BF16), vm((D, FF), BF16), vm((D, S), BF16),
                vm((4, FF, LN), F32), vm((4, S // 2, LN), U32), vm((_NSLOT, D, LN), U32),
                pltpu.SemaphoreType.DMA((cfg["nxc"] + 7,)), pltpu.SemaphoreType.DMA((cfg["nxc"],)),
            ],
            compiler_params=pltpu.CompilerParams(vmem_limit_bytes=120 * 1024 * 1024, flags=cfg["flags"] or None),
        )(np.zeros((256,), np.int32), A_x[0].T, A_wqkv, A_wo, B_w1, B_w2, B_w3, B_w4.T)
        return out.T[None]
    return run


pallas_interleave_layers__sliding_local_dilated__mixer_s_mlp__prompt_kernel = jax.jit(build(CFG))
```

```python
import functools

import jax
import jax.numpy as jnp
import numpy as np
import jax.experimental.pallas as pl
import jax.experimental.pallas.tpu as pltpu

S, D, NH, DH, FF = 2048, 448, 16, 28, 1792
WIN = 8
LN = 128
NT, HT = 16, 8
HD = D // 2
CG = D // 4
ROWS = 16
EPS = 1e-5
F32, BF16, U32 = jnp.float32, jnp.bfloat16, jnp.uint32
GELU_C = float(np.sqrt(2.0 / np.pi))
GELU_A = 0.044715 * GELU_C
GELU_K = float(np.cbrt(GELU_A))

PAIRS = [(0, 2), (4, 6), (1, 3), (5, 7), (8, 10), (12, 14), (9, 11), (13, 15)]

ORDER = """
q0 q1 q2 k1 v0 v1 q3 v2 v3 k0 k3 v4 k2 k5 o0 k4 v5 o3 o2 o1 h0 h1 h2 k6 h3 k7 s0 v7 q4 v6 s2 q5 q6 c0 a0 b0
e0 q7 a2 d0 e2 b2 c2 o4 o5 d2 o6 h5 h4 o7 k0 q0 h6 h7 s1 s3 v0 a1 b1 q2 c1 e1 s4 d1 k2 s6 c3 b3 a3 e3 v2 d3
q1 s5 c4 b4 a4 e4 d4 k1 v1 a6 b6 c6 e6 s7 d6 k3 v3 c5 a5 b5 q3 k4 e5 d5 a7 b7 c7 e7 v4 d7 o1 o0 k5 v5 o2 h0
h1 o3 h2 k6 h3 k7 v6 s0 v7 q4 s2 q6 q5 a0 b0 e0 a2 q7 c0 b2 c2 d0 o4 e2 o5 d2 o6 h4 h5 o7 s1 h6 h7 a1 s3 b1
c1 a3 e1 s4 d1 c3 b3 e3 s6 d3 a4 b4 c4 e4 d4 a6 s5 b6 c6 e6 s7 d6 a5 c5 b5 a7 e5 b7 e7 c7 d5 d7
"""

TUNE = dict(
    groups=(0, 3, 6, 9, 12), epilogue_lag=5, norm_lag=10, gather_lag=10, hold=22, early=2, out_span=150, gain=1.1,
    floor=0.7, cap=2.0, horizon=900, transpose_cost=11, w3_cost=8, q_cost=0.5, kv_cost=1.5, window_group=2,
    early_u=(4, 0), x_pins=(0, 1, 2, 3), prep_at={"o": 10, "1": 13, "2": 20, "3": 15, "4": 28}, x_at=6,
    waits={0: ("kv",), 6: (4, 5, 6, 7, "o", "1"), 13: ("3", "2", "4")})

QUEUED = {1: ("kv",), 3: (4, 5, 6, 7, "o", "1"), "kv": ("3", "2", "4")}

SLOT = {"qkv": 0, "wo": 11, "w1": 15, "w2": 19, "w3": 23, "w4": 37}
SLOTS = 50


def _neighbour(j, off):
    half, k = divmod(j, HT)
    step = (k + off) // HT
    other = half + step
    return half * HT + (k + off) % HT, step, other * HT + (k + off) % HT if step and 0 <= other < 2 else None


def _jobs(order):
    jobs = []
    for kind, p in order.split():
        for letter in "abce" if kind == "g" else kind:
            name = "qkv" if letter in "qkv" else "w3" if letter in "abce" else dict(o="wo", h="w1", s="w2", d="w4")[letter]
            chunk = tuple(group.index(letter) for group in ("qkv", "abce") if letter in group)
            jobs.append((name, int(p), int((name, int(p), 0) + chunk in jobs)) + chunk)
    return jobs


def _needs(item):
    kind, p, rnd = item[:3]
    if kind == "qkv":
        return [("norm", p, 0, "w4") if rnd else ("load", p, 0), ("prep", "qkv"[item[3]])]
    if kind == "attn":
        return [("qkv", p, rnd, 0)] + [("qkv", n, rnd, c) for n in (p & 6, p | 1) for c in (1, 2)]
    if kind == "shift":
        read = [t for j in PAIRS[p] for off in (-2, -1, 1, 2) for t in _neighbour(j, off)[::2]]
        return [("w1", n, rnd) for n, pair in enumerate(PAIRS) if any(j in read for j in pair)]
    return {"wo": [("attn", p, rnd)], "w1": [("norm", p, rnd, "wo")], "w2": [("shift", p, rnd)],
            "w3": [("norm", p, rnd, "w2")], "w4": [("w3", p, rnd, c) for c in range(4)]}[kind] + [("prep", kind[1])]


def _costs(task, tune):
    batch = [tune["transpose_cost"]]
    if task[0] == "prep":
        return {"o": [1] * 4 + batch + [1] * 14, "3": [tune["w3_cost"]] * 7, "4": [2] * 14}.get(
            task[1], batch + [1] * 14)
    if task[0] == "qkv":
        return [tune["kv_cost" if task[3] else "q_cost"]] * 7
    return {"load": ([1] if task[1] & 2 or PAIRS[task[1]][1] % HT // 2 < tune["early_u"][task[1] // 4] else batch) + [1] * 14, "norm": [1] * 14, "attn": [1] * 50,
            "shift": [1] * 14, "x_in": [batch[0] if f in tune["x_pins"] else 0 for f in range(4)], "x_out": batch * 4}.get(task[0], [1] * 7)


def _plan(order, tune):
    jobs = _jobs(order)
    points, first, count = [], {}, 0
    for job in jobs:
        first[job] = len(points)
        for i in range(7):
            n = len(points)
            for t in range(FF // 2 // LN if job[0] == "w4" else 2):
                if count % 4 == 0:
                    points += [(job, i, t, g) for g in tune["groups"]]
                count += 1
            if len(points) == n:
                points.append((job, i))
    end = len(points)
    after = dict(zip(jobs, [first[j] for j in jobs[1:]] + [end]))
    release, deadline, before = {}, {}, {}

    def visit(task, due):
        kind = task[0]
        if task not in deadline:
            before[task], release[task] = [], 0
            if kind in ("attn", "shift", "x_out"):
                before[task] = (_needs(task) if kind != "x_out"
                                else [("w4", p, 1) for p in range(4 * task[1], 4 * task[1] + 4)])
                release[task] = max(after[t] for t in before[task]) + tune["gather_lag"]
            elif kind == "norm":
                before[task] = [(task[3],) + task[1:3]]
                release[task] = after[before[task][0]] + tune["norm_lag"]
            elif kind == "prep":
                before[task] = [("prep", "qkv"["kvo".index(task[1])])] if task[1] in "kvo" else []
                release[task] = first[jobs[tune["prep_at"].get(task[1], 0)]]
            elif kind == "load":
                before[task] = [("load", task[1] - 2, 0)] if task[1] & 2 else [("x_in", task[1] // 4)]
            elif kind == "x_in":
                release[task] = first[jobs[tune["x_at"]]] if task[1] else 0
            else:
                release[task] = after[task] + tune["epilogue_lag"]
                if kind == "qkv" and task[3] > 0 and task[1] >= 4:
                    before[task] = [("qkv", task[1] - 4) + task[2:]]
                elif kind == "qkv" and task[3] == 2 and task[1] > 0:
                    before[task] = [("qkv", 0, task[2], 2)]
        deadline[task] = min(deadline.get(task, end), due)
        for t in before[task]:
            visit(t, deadline[task] - int(sum(_costs(task, tune))))

    for job in jobs:
        for t in _needs(job):
            visit(t, first[job] - tune["early"])
    for job in jobs:
        visit(job, min(end, after[job] + tune["hold"]))
    visit(("x_out", 0), max(after["w4", p, 1] for p in range(4)) + tune["out_span"])
    visit(("x_out", 1), end)
    rank = {t: (deadline[t], n) for n, t in enumerate(deadline)}
    left = {t: _costs(t, tune) for t in deadline}
    steps = []

    def emit(task, point):
        steps.append(("piece", task, point))
        return left[task].pop(0)

    def finish(task):
        for t in before[task]:
            finish(t)
        while left[task]:
            emit(task, None)

    finish(("prep", "q"))
    credit = 0.0
    for now, point in enumerate(points):
        job, i = point[:2]
        if now == first[job]:
            wait = [("wait", tune["waits"][jobs.index(job)])] if jobs.index(job) in tune["waits"] else []
            steps += wait if now else []
            for task in _needs(job):
                finish(task)
            steps += [] if now else wait
        if len(point) > 2:
            todo = sorted((t for t in left if left[t]), key=rank.get)
            rate, work = 0.0, 0
            for t in todo:
                work += sum(left[t])
                if deadline[t] - now <= tune["horizon"]:
                    rate = max(rate, work / max(deadline[t] - now, 1))
            credit += min(max(rate * tune["gain"], tune["floor"]), tune["cap"])
            while True:
                t = next((t for t in todo if left[t] and release[t] <= now and not any(left[b] for b in before[t])),
                         None)
                if t is None:
                    credit = min(credit, 1.0)
                if t is None or credit < left[t][0]:
                    break
                credit -= emit(t, point)
        if now + 1 == end or points[now + 1][:2] != (job, i):
            steps.append(("dot", job, i))
    for t in sorted(left, key=rank.get):
        finish(t)
    return steps


def _gelu_of_double(z):
    return z * jnp.tanh(z * (z * z * (8 * GELU_A) + 2 * GELU_C)) + z


def _gelu_scaled(z):
    return z * jnp.tanh(z * (z * z + GELU_C / GELU_K)) + z


def _lhs_operands(a11, a12, a21, a22):
    return a11 + a22, a21 + a22, a11, a22, a11 + a12, a21 - a11, a12 - a22


def _rhs_operands(b11, b12, b21, b22):
    return b11 + b22, b11, b12 - b22, b21 - b11, b22, b11 + b12, b21 + b22


def _combine(m1, m2, m3, m4, m5, m6, m7):
    return (m1 + m4) + (m7 - m5), m3 + m5, m2 + m4, (m1 - m2) + (m3 + m6)


def _mean(acc):
    return jnp.sum(acc, axis=0, keepdims=True) * (1.0 / D)


def _pad_rows(v, n):
    return v if v.shape[0] == n else jnp.concatenate([v, jnp.zeros((n - v.shape[0], v.shape[1]), v.dtype)], axis=0)


def _kernel(x_hbm, wqkv_hbm, wo_hbm, w1_hbm, w2_hbm, w3_hbm, w4_hbm, o_hbm,
            x_raw, wqkv_raw, wo_raw, w1_raw, w2_raw, w3_raw, w4_raw, o_raw, stage, tokens, weights, sem_in, sem_out,
            *, order, tune):
    steps = range(0, HD, ROWS)
    pieces = [steps[n:n + 2] for n in range(0, len(steps), 2)]
    zero = (jax.lax.broadcasted_iota(jnp.int32, (8, LN), 1) >> 7).astype(U32)

    def lanes(n):
        return jax.lax.broadcasted_iota(jnp.int32, (n, LN), 1)

    def bits(v):
        return pltpu.bitcast(v[:8, :LN], U32)

    def pinned(word, results):
        return word | (functools.reduce(jnp.bitwise_or, results) & zero)[:, :word.shape[1]]

    spans = [(r, min(LN, D - r)) for r in range(0, D, LN)]
    blocks = [(pl.ds(r, n), pl.ds(half * S // 2, S // 2)) for half in range(2) for r, n in spans]
    q_cols, kv_cols = pl.ds(0, 4 * LN), pl.ds(4 * LN, 3 * D - 4 * LN)
    sources = [(c, x_hbm.at[blk], x_raw.at[blk]) for c, blk in enumerate(blocks)] + [
        ("q", wqkv_hbm.at[:, q_cols], wqkv_raw.at[:, q_cols]), ("kv", wqkv_hbm.at[:, kv_cols], wqkv_raw.at[:, kv_cols]),
        ("o", wo_hbm, wo_raw), ("1", w1_hbm, w1_raw), ("2", w2_hbm, w2_raw), ("3", w3_hbm, w3_raw),
        ("4", w4_hbm, w4_raw)]
    loads = {name: pltpu.make_async_copy(src, dst, sem_in.at[n]) for n, (name, src, dst) in enumerate(sources)}
    stores = [pltpu.make_async_copy(o_raw.at[blk], o_hbm.at[blk], sem_out.at[c]) for c, blk in enumerate(blocks)]

    landed = set()

    def arrived(name):
        landed.add(name)
        loads[name].wait()
        for queued in QUEUED.get(name, ()):
            loads[queued].start()

    def lhs_tiles(name, c, i):
        k = FF // 2 if name == "w4" else HD
        n = pl.cdiv(k, LN)
        units = [(c * 7 + i) * n + t for t in range(n)]
        return [(SLOT[name] + u // 4, u % 4 * (HD // 2), pl.ds(0, min(LN, k - t * LN))) for t, u in enumerate(units)]

    def put_words(name, c, i, r, words):
        for t, (slot, r0, w) in enumerate(lhs_tiles(name, c, i)):
            weights[slot, pl.ds(r0 + r, words.shape[0]), w] = words[:, t * LN:t * LN + w.size]

    def put_lhs(name, c, r, quadrants, exact=None):
        words = [pltpu.bitcast(exact[i] if exact and i in exact else v.astype(BF16), U32)
                 for i, v in enumerate(_lhs_operands(*quadrants))]
        for i, u in enumerate(words):
            put_words(name, c, i, r // 2, u)
        return [u[:8, :LN] for u in words[5:]]

    def get_lhs(name, c, i, pins):
        cols = []
        for t, (slot, r0, w) in enumerate(lhs_tiles(name, c, i)):
            parts, r = [], 0
            for g in sorted(g for tile, g in pins if tile == t):
                if 8 * g > r:
                    parts.append(weights[slot, pl.ds(r0 + r, 8 * g - r), w])
                parts.append(pinned(weights[slot, pl.ds(r0 + 8 * g, 8), w], pins[t, g]))
                r = 8 * g + 8
            if r < HD // 2:
                parts.append(weights[slot, pl.ds(r0 + r, HD // 2 - r), w])
            cols.append(jnp.concatenate(parts, axis=0))
        return pltpu.bitcast(jnp.concatenate(cols, axis=1), BF16)

    def put_halves(name, k):
        for r in steps:
            yield put_lhs(name, 0, r, [v[o + r:o + r + ROWS] for o in (0, HD) for v in k])

    def prepare_qkv(c):
        if c == 0:
            arrived("q")
        for b in ((0, 1, 2, 3), (4, 5, 6), (7, 8, 9, 10))[c]:
            n = min(LN, 3 * D - b * LN)
            t = [_pad_rows(wqkv_raw[pl.ds(h * HD, HD), pl.ds(b * LN, n)], 2 * LN).T.astype(F32) for h in range(2)]
            for h in range(4):
                stage[h, pl.ds(b * LN, n), :] = t[h // 2][:, h % 2 * LN:(h % 2 + 1) * LN]
        yield [bits(v[-8:]) for v in t]
        for d in range(DH // 2):
            heads = [pl.ds(c * D + dd, NH, stride=DH) for dd in (d, d + DH // 2)]
            yield put_lhs("qkv", c, d * NH, [
                jnp.concatenate([stage[2 * h, rows, :], stage[2 * h + 1, rows, :][:, :HD - LN]], axis=1)
                for rows in heads for h in range(2)])

    def prepare_o():
        for c, (col, n) in enumerate(spans):
            w = wo_raw[:, pl.ds(col, n)].astype(F32)
            w = w if n == LN else jnp.concatenate([w, jnp.zeros((D, LN - n), F32)], axis=1)
            stage[c, pl.ds(0, D), :] = w
            yield [bits(w[-8:])]
        k = [[], []]
        for c, (_, n) in enumerate(spans):
            for h in range(2):
                rows = [stage[c, pl.ds(d, NH, stride=DH), :] for d in range(h * DH // 2, (h + 1) * DH // 2)]
                k[h].append(jnp.concatenate(rows, axis=0)[:, :n].astype(BF16).T.astype(F32))
        yield [bits(v[-8:]) for half in k for v in half]
        yield from put_halves("wo", [jnp.concatenate(v, axis=0) for v in k])

    def prepare_square(name, raw):
        k = [[raw[pl.ds(h * HD, HD), pl.ds(col, n)].T.astype(F32) for h in range(2)] for col, n in spans]
        yield [bits(v[-8:]) for both in k for v in both]
        yield from put_halves(name, [jnp.concatenate([v[h] for v in k], axis=0) for h in range(2)])

    def prepare_3():
        for b in range(FF // 2 // LN):
            done = []
            for i, v in enumerate(_lhs_operands(*[w3_raw[pl.ds(h * HD, HD), pl.ds(m + b * LN, LN)].astype(F32)
                                                  for m in (0, FF // 2) for h in range(2)])):
                words = pltpu.bitcast(v.astype(BF16).T, U32)
                c, at = divmod(b * LN // 2, HD // 2)
                n = min(HD // 2 - at, LN // 2)
                put_words("w3", c, i, at, words[:n])
                if n < LN // 2:
                    put_words("w3", c + 1, i, 0, words[n:])
                done.append(words[-8:, :LN])
            yield done

    def prepare_4():
        for r in steps:
            raw = [w4_raw[pl.ds(o + r, ROWS), pl.ds(k, FF // 2)] for o in (0, HD) for k in (0, FF // 2)]
            yield put_lhs("w4", 0, r, [v.astype(F32) for v in raw], exact={2: raw[0], 3: raw[3]})

    act, rhs_rows, rhs = {}, {}, {}

    def rows_of(name, tile, r, n):
        if n < ROWS:
            return act[name, tile, r - r % ROWS][r % ROWS:r % ROWS + n]
        return jnp.concatenate([act[name, tile, k] for k in range(r, r + n, ROWS)], axis=0)

    def quad(p, r):
        return [(j, o + r) for o in (0, HD) for j in PAIRS[p]]

    def put_rhs(name, p, r, quadrants):
        rows = rhs_rows.setdefault((name, p), {})
        ops = rows[r] = _rhs_operands(*quadrants)
        if len(rows) * ROWS == (FF // 2 if name == "w4" else HD):
            rhs[name, p] = [jnp.concatenate([rows[k][i] for k in sorted(rows)], axis=0).astype(BF16) for i in range(7)]
            del rhs_rows[name, p]
        return [bits(ops[2]), bits(ops[3])]

    def accumulate(sums, i, v):
        s = functools.reduce(jnp.add, [v[r:r + 8] for r in range(0, v.shape[0], 8)])
        sums[i % 2] = s if sums[i % 2] is None else sums[i % 2] + s

    early, finished = {}, {}

    def token_rows(u):
        return pl.ds(u // (HT // 2) * (S // 4) + u % (HT // 2), LN, stride=HT // 2)

    def x_in(half):
        for f, (r, n) in enumerate(spans):
            if half == 0:
                arrived(f)
            for t in range(half * HT, (half + 1) * HT):
                words = pltpu.bitcast(_pad_rows(x_raw[pl.ds(r, n), pl.ds(t * LN, LN)], LN).T, U32)
                tokens[f, pl.ds(t * LN // 2, LN // 2), :] = words
            done = [words[-8:]]
            for u in range(half * HT // 2, half * HT // 2 + tune["early_u"][half]):
                early[u, f] = tokens[f, token_rows(u), :].T[:n]
                done = [early[u, f][-8:]]
            yield done if half == 0 or f in tune["x_pins"] else []

    def load(p):
        sums = [None, None]
        for i, j in enumerate(PAIRS[p]):
            if j % 2 == 0:
                w = jnp.concatenate([early[j // 2, f] if (j // 2, f) in early
                                     else tokens[f, token_rows(j // 2), :].T[:n] for f, (_, n) in enumerate(spans)], axis=0)
                for odd, x in enumerate((w << 16, w & np.uint32(0xFFFF0000))):
                    x = pltpu.bitcast(x, F32)
                    act.update({("x", j + odd, r): x[r:r + ROWS] for r in range(0, D, ROWS)})
            accumulate(sums, i, rows_of("x", j, 0, D))
        yield [bits(v) for v in sums]
        yield from normalise("x", p, sums, lambda var, rstd: rstd, "qkv")

    def unload(j):
        finished[j] = pltpu.bitcast(rows_of("x", j, 0, D).astype(BF16).astype(F32), U32)
        if j ^ 1 not in finished:
            return []
        w = (finished[j & ~1] >> 16) | finished[j | 1]
        for f, (r, n) in enumerate(spans):
            words = _pad_rows(w[r:r + n], LN).T
            tokens[f, token_rows(j // 2), :] = words
        return [words[-8:]]

    def x_out(half):
        for f, (r, n) in enumerate(spans):
            for t in range(half * HT, (half + 1) * HT):
                x = pltpu.bitcast(tokens[f, pl.ds(t * LN // 2, LN // 2), :], BF16).T
                o_raw[pl.ds(r, n), pl.ds(t * LN, LN)] = x[:n]
            stores[half * len(spans) + f].start()
            yield [pltpu.bitcast(x, U32)[:8]]

    norms, first_norm = {}, {}

    def normalise(src, p, sums, gain, name, keep=None):
        mean, acc = [_mean(v) for v in sums], [None, None]
        for piece in pieces:
            for r in piece:
                for i, at in enumerate(quad(p, r)):
                    xc = act[(src,) + at] - mean[i % 2]
                    accumulate(acc, i, xc * xc)
            yield [bits(v) for v in acc]
        var = [_mean(v) for v in acc]
        rstd = [jax.lax.rsqrt(v + EPS) for v in var]
        if keep is not None:
            keep[p] = mean, rstd
        scale = [gain(v, r) for v, r in zip(var, rstd)]
        for piece in pieces:
            yield [v for r in piece for v in put_rhs(
                name, p, r, [(act[(src,) + at] - mean[i % 2]) * scale[i % 2] for i, at in enumerate(quad(p, r))])]

    def after_qkv(p, c, out):
        name = "qkv"[c]
        for piece in pieces:
            for r in piece:
                quadrants = out(r)
                for (j, at), t in zip(quad(p, r), quadrants):
                    act[name, (j, 0), at] = t
                    for by in () if c == 0 else (1, 2) if j % HT >= 2 else (1,):
                        if j >= HT:
                            earlier = pltpu.roll(jnp.where(lanes(ROWS) >= LN - by, act[name, (j - HT, 0), at], t), by, 1)
                        else:
                            earlier = pltpu.roll(t, by, 1)
                            if c == 2:
                                token0 = jnp.broadcast_to(act["v", (0, 0), at][:, :1], t.shape)
                                earlier = jnp.where(lanes(ROWS) < by, token0, earlier)
                        act[name, (j, by), at] = earlier
            yield [bits(quadrants[0][-8:]), bits(quadrants[3][-8:])]

    def attention(p):
        a = PAIRS[p][0]
        window = [(a // HT * HT + (a + 2 * i - 14) % HT, -((a % HT + 2 * i - 14) // HT)) for i in range(WIN + 1)]
        prob = {}
        for heads in (0, 8):
            logit = {}
            for i0 in range(0, WIN + 1, tune["window_group"]):
                entries = range(i0, min(i0 + tune["window_group"], WIN + 1))
                use = [(t, i) for i in entries for t in range(2) if 0 <= i - t < WIN]
                acc = {}
                for d in range(DH):
                    q = [rows_of("q", (a + 2 * t, 0), d * NH + heads, 8) for t in range(2)]
                    k = {i: rows_of("k", window[i], d * NH + heads, 8) for i in entries}
                    for t, i in use:
                        acc[t, i] = acc[t, i] + q[t] * k[i] if d else q[t] * k[i]
                    if d + 1 in [DH * (n + 1) // len(entries) for n in range(len(entries))]:
                        yield [bits(acc[u]) for u in use]
                for t, i in use:
                    lg = acc[t, i] * (DH ** -0.5)
                    logit[t, i - t] = jnp.where(lanes(8) < window[i][1], -1e9, lg) if a < HT and window[i][1] else lg
            for t in range(2):
                lg = [logit[t, i] for i in range(WIN)]
                peak = functools.reduce(jnp.maximum, lg)
                e = [jnp.exp(v - peak) for v in lg]
                inv = 1.0 / functools.reduce(jnp.add, e)
                prob[t, heads] = [v * inv for v in e]
                yield [bits(inv)]
        for d in range(DH // 2):
            out = []
            for heads in (0, 8):
                out.append([])
                for dd in (d, d + DH // 2):
                    v = [rows_of("v", entry, dd * NH + heads, 8) for entry in window]
                    out[-1] += [functools.reduce(jnp.add, [prob[t, heads][i] * v[i + t] for i in range(WIN)])
                                for t in range(2)]
                if heads == 0:
                    yield [bits(v) for v in out[0][1:3]]
            yield put_rhs("wo", p, d * NH, [jnp.concatenate(v, axis=0) for v in zip(*out)])

    def update(p, out, dst, fn):
        sums = [None, None]
        for piece in pieces:
            for r in piece:
                for i, (at, t) in enumerate(zip(quad(p, r), out(r))):
                    act[(dst,) + at] = fn(i % 2, at, t)
                    accumulate(sums, i, act[(dst,) + at])
            yield sums

    def after_wo(p, out):
        for sums in update(p, out, "x", lambda i, at, t: act[("x",) + at] + t):
            norms[p, "wo"] = normalise(
                "x", p, sums, lambda var, rstd: 0.5 * rstd * jax.lax.rsqrt(var * rstd * rstd + EPS), "w1", first_norm)
            yield [bits(v) for v in sums]

    def after_w1(p, out):
        for piece in pieces:
            for r in piece:
                hidden = [_gelu_of_double(t) for t in out(r)]
                act.update({("h",) + at: h for at, h in zip(quad(p, r), hidden)})
            yield [bits(h[-8:]) for h in hidden]

    def shifted(j, off, r):
        tile, step, other = _neighbour(j, off)
        h = act["h", tile, r]
        if step:
            edge = 0.0 if other is None else act["h", other, r]
            h = pltpu.roll(jnp.where(lanes(ROWS) == (0 if step > 0 else LN - 1), edge, h), -step % LN, 1)
        return h

    def shift(p):
        for r in steps:
            offsets = ((-1, -2), (1, 2))[r // CG]
            yield put_rhs("w2", p, r, [shifted(j, off, o + r) for off, o in zip(offsets, (0, HD)) for j in PAIRS[p]])

    def after_w2(p, out):
        mean, rstd = first_norm[p]
        for sums in update(p, out, "x1", lambda i, at, t: (act[("x",) + at] - mean[i]) * rstd[i] + t):
            norms[p, "w2"] = normalise("x1", p, sums, lambda var, rstd: GELU_K * rstd, "w3")
            yield [bits(v) for v in sums]

    def after_w3(p, c, out):
        for piece in pieces:
            yield [v for r in piece for v in put_rhs("w4", p, c * HD + r, [_gelu_scaled(t) for t in out(r)])]

    def after_w4(p, last, out):
        def residual(i, at, t):
            return act[("x",) + at] + (act[("x1",) + at] + t * (0.5 / GELU_K))

        for n, sums in enumerate(update(p, out, "x", residual)):
            if not last:
                norms[p, "w4"] = normalise("x", p, sums, lambda var, rstd: rstd, "qkv")
            yield ([v for j in PAIRS[p] for v in unload(j)] if last and n + 1 == len(pieces)
                   else [bits(v) for v in sums])

    products, pins, running = {}, {}, {}

    def start(task):
        kind, p = task[:2]
        assert kind != "x_in" or p == 0 or landed >= set(range(4, 8))
        if kind == "prep":
            assert p == "q" or ("kv" if p in "kv" else p) in landed
            if p in "qkv":
                return prepare_qkv("qkv".index(p))
            return {"o": prepare_o, "1": lambda: prepare_square("w1", w1_raw), "2": lambda: prepare_square("w2", w2_raw),
                    "3": prepare_3, "4": prepare_4}[p]()
        if kind == "norm":
            return norms.pop((p, task[3]))
        if task not in products:
            return {"load": load, "attn": attention, "shift": shift, "x_in": x_in, "x_out": x_out}[kind](p)
        m = products.pop(task)

        def out(r):
            return _combine(*[v[r:r + ROWS] for v in m])

        if kind in ("qkv", "w3"):
            return (after_qkv if kind == "qkv" else after_w3)(p, task[3], out)
        if kind == "w4":
            return after_w4(p, task[2] == 1, out)
        return {"wo": after_wo, "w1": after_w1, "w2": after_w2}[kind](p, out)

    for name in ("q", 0, 1, 2, 3):
        loads[name].start()
    for step in _plan(order, tune):
        if step[0] == "wait":
            for name in step[1]:
                arrived(name)
        elif step[0] == "piece":
            _, task, point = step
            if task not in running:
                running[task] = start(task)
            results = next(running[task])
            if point is not None and results and task[0] != "qkv":
                pins.setdefault(point[:2], {}).setdefault(point[2:], []).extend(results)
        else:
            _, job, i = step
            w = get_lhs(job[0], job[3] if len(job) > 3 else 0, i, pins.pop((job, i), {}))
            products.setdefault(job, []).append(jnp.dot(w, rhs[job[:2]][i], preferred_element_type=F32))
    assert landed == set(loads) and all(next(task, None) is None for task in running.values())
    for copy in stores:
        copy.wait()


def _run(A_x, A_wqkv, A_wo, B_w1, B_w2, B_w3, B_w4, order=None, tune=None):
    vmem = pltpu.VMEM
    out = pl.pallas_call(
        functools.partial(_kernel, order=order or ORDER, tune=tune or TUNE),
        out_shape=jax.ShapeDtypeStruct((D, S), BF16),
        in_specs=[pl.BlockSpec(memory_space=pl.ANY)] * 7,
        out_specs=pl.BlockSpec(memory_space=pl.ANY),
        scratch_shapes=[
            vmem((D, S), BF16), vmem((D, 3 * D), BF16), vmem((D, D), BF16), vmem((D, D), BF16), vmem((D, D), BF16),
            vmem((D, FF), BF16), vmem((D, FF), BF16), vmem((D, S), BF16),
            vmem((4, FF, LN), F32), vmem((4, S // 2 + 8, LN), U32), vmem((SLOTS, D, LN), U32),
            pltpu.SemaphoreType.DMA((15,)), pltpu.SemaphoreType.DMA((8,)),
        ],
        compiler_params=pltpu.CompilerParams(vmem_limit_bytes=120 * 1024 * 1024),
    )(A_x[0].T, A_wqkv, A_wo, B_w1, B_w2, B_w3, B_w4.T)
    return out.T[None]


@jax.jit
def pallas_interleave_layers__sliding_local_dilated__mixer_s_mlp__prompt_kernel(
    A_x: jax.Array,
    A_wqkv: jax.Array,
    A_wo: jax.Array,
    B_x: jax.Array,
    B_w1: jax.Array,
    B_w2: jax.Array,
    B_w3: jax.Array,
    B_w4: jax.Array,
):
    del B_x
    return _run(A_x, A_wqkv, A_wo, B_w1, B_w2, B_w3, B_w4)
```
